```python
import jax
import jax.numpy as jnp

def _softmax(x, axis=-1):
    return jax.nn.softmax(x, axis=axis)
def _gelu(x):
    return jax.nn.gelu(x, approximate=True)
def _silu(x):
    return jax.nn.silu(x)
def _sigmoid(x):
    return jax.nn.sigmoid(x)
def _layernorm(x, axis=-1, eps=1e-5):
    m = jnp.mean(x, axis=axis, keepdims=True)
    v = jnp.var(x, axis=axis, keepdims=True)
    return (x - m) / jnp.sqrt(v + eps)
def _scatter_add(tgt, idx, src, axis=0):
    return tgt.at[idx].add(src)
def _segment_sum(src, seg, n):
    return jax.ops.segment_sum(src, seg, n)
class _Rng:
    def __init__(self, key):
        self._k = key
    def _next(self):
        self._k, sub = jax.random.split(self._k)
        return sub
    def normal(self, shape):
        return jax.random.normal(self._next(), shape, dtype=jnp.bfloat16)
    def randint(self, lo, hi, shape):
        return jax.random.randint(self._next(), shape, lo, hi, dtype=jnp.int32)
    def uniform(self, shape, lo=0.0, hi=1.0):
        return jax.random.uniform(self._next(), shape, jnp.bfloat16, lo, hi)
    def permutation(self, n):
        return jax.random.permutation(self._next(), n)


kernel_name = 'interleave_layers__sliding_local_dilated__glu_gated_bilinear__prompt'

def setup_inputs():
    _rng = _Rng(jax.random.key(int.from_bytes(__import__("os").urandom(4), "little")))
    _w = (lambda a: (lambda t: t.astype(jnp.bfloat16) if jnp.issubdtype(t.dtype, jnp.floating) else t)(jnp.asarray(a)))
    def _A_setup():
        B, S, D = 1, 2048, 576
        return {
            "x": _w((lambda *s: _rng.normal(s) * 0.05)(B, S, D)),
            "wqkv": _w((lambda *s: _rng.normal(s) * 0.05)(D, 3 * D)),
            "wo": _w((lambda *s: _rng.normal(s) * 0.05)(D, D)),
        }
    _A_in = _A_setup()

    def _B_setup():
        B, S, D, F = 1, 2048, 576, 4608
        return {
            "x": _w((lambda *s: _rng.normal(s) * 0.05)(B, S, D)),
            "w_gate": _w((lambda *s: _rng.normal(s) * 0.05)(D, F) * (D ** -0.5)),
            "w_up": _w((lambda *s: _rng.normal(s) * 0.05)(D, F) * (D ** -0.5)),
            "w_down": _w((lambda *s: _rng.normal(s) * 0.05)(F, D) * (F ** -0.5)),
        }
    _B_in = _B_setup()

    return {
        "A_x": _A_in["x"],
        "A_wqkv": _A_in["wqkv"],
        "A_wo": _A_in["wo"],
        "B_x": _B_in["x"],
        "B_w_gate": _B_in["w_gate"],
        "B_w_up": _B_in["w_up"],
        "B_w_down": _B_in["w_down"],
    }

def reference(A_x, A_wqkv, A_wo, B_x, B_w_gate, B_w_up, B_w_down):
    def _A_ref(x, wqkv, wo):
        B, S, D = x.shape
        H = 32; Dh = D // H
        W, dil = 8, 2
        qkv = (lambda x, *d: x.transpose(*d))((x @ wqkv).reshape(B, S, 3, H, Dh), 2, 0, 3, 1, 4)
        q, k, v = qkv[0], qkv[1], qkv[2]
        scale = Dh ** -0.5
        pos = jnp.arange(S)
        off = jnp.arange(W) * dil
        idx = pos[:, None] - off[None, :]
        mask = idx >= 0
        idx_c = jnp.where(mask, idx, 0).reshape(-1)
        kg = k[:, :, idx_c, :].reshape(B, H, S, W, Dh)
        vg = v[:, :, idx_c, :].reshape(B, H, S, W, Dh)
        logits = jnp.einsum("bhsd,bhswd->bhsw", q, kg) * scale
        logits = jnp.where(mask[None, None, :, :], logits, -1e9)
        attn = _softmax(logits, axis=-1)
        o = jnp.einsum("bhsw,bhswd->bhsd", attn, vg)
        return (lambda x, *d: x.transpose(*d))(o, 0, 2, 1, 3).reshape(B, S, D) @ wo

    def _B_ref(x, w_gate, w_up, w_down):
        g = jnp.einsum("bsd,df->bsf", x, w_gate)
        u = jnp.einsum("bsd,df->bsf", x, w_up)
        h = g * u
        return jnp.einsum("bsf,fd->bsd", h, w_down)

    x = A_x
    x = x + _A_ref(_layernorm(x, axis=-1), A_wqkv, A_wo)
    x = x + _B_ref(_layernorm(x, axis=-1), B_w_gate, B_w_up, B_w_down)
    x = x + _A_ref(_layernorm(x, axis=-1), A_wqkv, A_wo)
    x = x + _B_ref(_layernorm(x, axis=-1), B_w_gate, B_w_up, B_w_down)
    return x
```

```python
import functools
import jax
import jax.numpy as jnp
import jax.experimental.pallas as pl
import jax.experimental.pallas.tpu as pltpu

TM = 512
FC = 512
RC = 64
HALO = 16
W, DIL = 8, 2
D, H, DH = 576, 32, 18
BF = jnp.bfloat16
F32 = jnp.float32


def _ln(x):
    m = jnp.mean(x, axis=-1, keepdims=True)
    xc = x - m
    v = jnp.mean(xc * xc, axis=-1, keepdims=True)
    return (xc * jax.lax.rsqrt(v + 1e-5)).astype(BF)


def _kernel(x_ref, wqkv_ref, wo_ref, wg_hbm, wu_hbm, wd_hbm, o_ref,
            wg, wu, wd, kv, halo, obuf, sems, *, nf):
    i = pl.program_id(0)

    def copies(c):
        cs = pl.ds(c * FC, FC)
        return (pltpu.make_async_copy(wg_hbm.at[:, cs], wg.at[:, cs], sems.at[0, c]),
                pltpu.make_async_copy(wu_hbm.at[:, cs], wu.at[:, cs], sems.at[1, c]),
                pltpu.make_async_copy(wd_hbm.at[cs, :], wd.at[cs, :], sems.at[2, c]))

    @pl.when(i == 0)
    def _():
        for c in range(nf):
            for cp in copies(c):
                cp.start()
        halo[...] = jnp.zeros(halo.shape, F32)

    scale = DH ** -0.5

    def attn(x, layer):
        qkv = jnp.dot(_ln(x), wqkv_ref[...], preferred_element_type=F32)
        t = lambda j: qkv[:, j * 128:(j + 1) * 128]
        kv[0:HALO, :] = halo[layer]
        for j in range(4):
            kv[HALO:, j * 128:(j + 1) * 128] = t(4 + j)
            kv[HALO:, (5 + j) * 128:(6 + j) * 128] = t(8 + j)
        kv[HALO:, 512:640] = t(13)
        kv[HALO:, 1152:1280] = t(12)
        halo[layer] = kv[TM:TM + HALO, :]
        for r in range(TM // RC):
            r0 = r * RC
            q = [qkv[r0:r0 + RC, j * 128:(j + 1) * 128] for j in (0, 1, 2, 3, 12)]
            lg = []
            for w in range(W):
                s = HALO + r0 - DIL * w
                p = None
                for j in range(5):
                    e = q[j] * kv[s:s + RC, j * 128:(j + 1) * 128]
                    p = e if p is None else p + e
                p = p + pltpu.roll(p, 64, 1)
                p = (p + pltpu.roll(p, 32, 1)) * scale
                if r0 < DIL * w:
                    pos = i * TM + r0 + jax.lax.broadcasted_iota(jnp.int32, (RC, 128), 0)
                    p = jnp.where(pos >= DIL * w, p, -1e9)
                lg.append(p)
            m = functools.reduce(jnp.maximum, lg)
            ex = [jnp.exp(p - m) for p in lg]
            inv = 1.0 / functools.reduce(jnp.add, ex)
            for j in range(5):
                acc = None
                for w in range(W):
                    s = HALO + r0 - DIL * w
                    e = ex[w] * kv[s:s + RC, (5 + j) * 128:(6 + j) * 128]
                    acc = e if acc is None else acc + e
                obuf[r0:r0 + RC, j * 128:(j + 1) * 128] = (acc * inv).astype(BF)
        return x + jnp.dot(obuf[...], wo_ref[...], preferred_element_type=F32)

    def ffn(x, first):
        xn = _ln(x)
        acc = x
        for c in range(nf):
            if first:
                @pl.when(i == 0)
                def _():
                    for cp in copies(c):
                        cp.wait()
            cs = slice(c * FC, (c + 1) * FC)
            g = jnp.dot(xn, wg[:, cs], preferred_element_type=F32)
            u = jnp.dot(xn, wu[:, cs], preferred_element_type=F32)
            acc = acc + jnp.dot((g * u).astype(BF), wd[cs, :], preferred_element_type=F32)
        return acc

    x = x_ref[...].astype(F32)
    x = attn(x, 0)
    x = ffn(x, True)
    x = attn(x, 1)
    x = ffn(x, False)
    o_ref[...] = x.astype(o_ref.dtype)


@jax.jit
def pallas_interleave_layers__sliding_local_dilated__glu_gated_bilinear__prompt_kernel(
        A_x, A_wqkv, A_wo, B_x, B_w_gate, B_w_up, B_w_down):
    Bn, S, _ = A_x.shape
    F = B_w_gate.shape[1]
    nf = F // FC
    x = A_x.reshape(Bn * S, D)
    wp = A_wqkv.reshape(D, 3, H, DH).transpose(0, 1, 3, 2).reshape(D, 3, D)
    z = jnp.zeros((D, 64), wp.dtype)
    wq = jnp.concatenate([wp[:, 0, :512], wp[:, 1, :512], wp[:, 2, :512],
                          wp[:, 0, 512:], wp[:, 2, 512:], wp[:, 1, 512:], z], axis=1)
    wop = A_wo.reshape(H, DH, D).transpose(1, 0, 2).reshape(D, D)
    wo = jnp.concatenate([wop[:512], jnp.zeros((64, D), wop.dtype), wop[512:]], axis=0)
    anyspec = pl.BlockSpec(memory_space=pl.ANY)
    out = pl.pallas_call(
        functools.partial(_kernel, nf=nf),
        grid=(S // TM,),
        in_specs=[pl.BlockSpec((TM, D), lambda i: (i, 0)),
                  pl.BlockSpec((D, 1792), lambda i: (0, 0)),
                  pl.BlockSpec((640, D), lambda i: (0, 0)),
                  anyspec, anyspec, anyspec],
        out_specs=pl.BlockSpec((TM, D), lambda i: (i, 0)),
        out_shape=jax.ShapeDtypeStruct((S, D), A_x.dtype),
        scratch_shapes=[pltpu.VMEM((D, F), BF), pltpu.VMEM((D, F), BF), pltpu.VMEM((F, D), BF),
                        pltpu.VMEM((TM + HALO, 1280), F32), pltpu.VMEM((2, HALO, 1280), F32),
                        pltpu.VMEM((TM, 640), BF),
                        pltpu.SemaphoreType.DMA((3, nf))],
        compiler_params=pltpu.CompilerParams(dimension_semantics=("arbitrary",),
                                             vmem_limit_bytes=100 * 1024 * 1024),
    )(x, wq, wo, B_w_gate, B_w_up, B_w_down)
    return out.reshape(Bn, S, D)
```

```python
import functools
import jax
import jax.numpy as jnp
import jax.experimental.pallas as pl
import jax.experimental.pallas.tpu as pltpu

TM = 512
FC = 512
RC = 64
HALO = 16
W, DIL = 8, 2
D, H, DH = 576, 32, 18
BF = jnp.bfloat16
F32 = jnp.float32


def _ln(x):
    m = jnp.mean(x, axis=-1, keepdims=True)
    xc = x - m
    v = jnp.mean(xc * xc, axis=-1, keepdims=True)
    return (xc * jax.lax.rsqrt(v + 1e-5)).astype(BF)


def _kernel(x_ref, wqkv_in, wo_in, wg_hbm, wu_hbm, wd_hbm, o_ref,
            wqkv_ref, wo_ref, wg, wu, wd, kv, halo, obuf, sems, *, nf):
    i = pl.program_id(0)

    def copies(c):
        cs = pl.ds(c * FC, FC)
        return (pltpu.make_async_copy(wg_hbm.at[:, cs], wg.at[:, cs], sems.at[0, c]),
                pltpu.make_async_copy(wu_hbm.at[:, cs], wu.at[:, cs], sems.at[1, c]),
                pltpu.make_async_copy(wd_hbm.at[:, cs], wd.at[:, cs], sems.at[2, c]))

    @pl.when(i == 0)
    def _():
        for c in range(nf):
            for cp in copies(c):
                cp.start()
        halo[...] = jnp.zeros(halo.shape, F32)
        lane = jax.lax.broadcasted_iota(jnp.int32, (640, 128), 1)
        row = jax.lax.broadcasted_iota(jnp.int32, (640, 128), 0)

        def part(sec, n0, lo, hi):
            t0 = {0: 0, 1: 4, 2: 9}[sec] * 128
            n = n0 + lane - lo
            src = (n % H) * DH + n // H + (sec * D - t0)
            ok = (src == row) & (lane >= lo) & (lane < hi)
            wid = min(640, 3 * D - t0)
            P = jnp.where(ok, 1.0, 0.0).astype(BF)[:wid]
            return jnp.dot(wqkv_in[:, t0:t0 + wid], P, preferred_element_type=F32)

        for sec in range(3):
            for j in range(4):
                c = (sec * 4 + j) * 128
                wqkv_ref[:, c:c + 128] = part(sec, j * 128, 0, 128).astype(BF)
        wqkv_ref[:, 1536:1664] = (part(0, 512, 0, 64) + part(2, 512, 64, 128)).astype(BF)
        wqkv_ref[:, 1664:1792] = part(1, 512, 0, 64).astype(BF)
        r = jax.lax.broadcasted_iota(jnp.int32, (640, D), 0)
        cc = jax.lax.broadcasted_iota(jnp.int32, (640, D), 1)
        n = jnp.where(r >= 576, r - 64, r)
        ok = ((n % H) * DH + n // H == cc) & ((r < 512) | (r >= 576))
        wo_ref[...] = jnp.dot(jnp.where(ok, 1.0, 0.0).astype(BF), wo_in[...],
                              preferred_element_type=F32).astype(BF)

    scale = DH ** -0.5

    def attn(x, layer):
        qkv = jnp.dot(_ln(x), wqkv_ref[...], preferred_element_type=F32)
        t = lambda j: qkv[:, j * 128:(j + 1) * 128]
        kv[0:HALO, :] = halo[layer]
        for j in range(4):
            kv[HALO:, j * 128:(j + 1) * 128] = t(4 + j)
            kv[HALO:, (5 + j) * 128:(6 + j) * 128] = t(8 + j)
        kv[HALO:, 512:640] = t(13)
        kv[HALO:, 1152:1280] = t(12)
        halo[layer] = kv[TM:TM + HALO, :]
        for r in range(TM // RC):
            r0 = r * RC
            q = [qkv[r0:r0 + RC, j * 128:(j + 1) * 128] for j in (0, 1, 2, 3, 12)]
            lg = []
            for w in range(W):
                s = HALO + r0 - DIL * w
                p = None
                for j in range(5):
                    e = q[j] * kv[s:s + RC, j * 128:(j + 1) * 128]
                    p = e if p is None else p + e
                p = p + pltpu.roll(p, 64, 1)
                p = (p + pltpu.roll(p, 32, 1)) * scale
                if r0 < DIL * w:
                    pos = i * TM + r0 + jax.lax.broadcasted_iota(jnp.int32, (RC, 128), 0)
                    p = jnp.where(pos >= DIL * w, p, -1e9)
                lg.append(p)
            m = functools.reduce(jnp.maximum, lg)
            ex = [jnp.exp(p - m) for p in lg]
            inv = 1.0 / functools.reduce(jnp.add, ex)
            for j in range(5):
                acc = None
                for w in range(W):
                    s = HALO + r0 - DIL * w
                    e = ex[w] * kv[s:s + RC, (5 + j) * 128:(6 + j) * 128]
                    acc = e if acc is None else acc + e
                obuf[r0:r0 + RC, j * 128:(j + 1) * 128] = (acc * inv).astype(BF)
        return x + jnp.dot(obuf[...], wo_ref[...], preferred_element_type=F32)

    def ffn(x, first):
        xn = _ln(x)
        acc = x
        for c in range(nf):
            if first:
                @pl.when(i == 0)
                def _():
                    for cp in copies(c):
                        cp.wait()
            cs = slice(c * FC, (c + 1) * FC)
            g = jnp.dot(xn, wg[:, cs], preferred_element_type=F32)
            u = jnp.dot(xn, wu[:, cs], preferred_element_type=F32)
            acc = acc + jax.lax.dot_general((g * u).astype(BF), wd[:, cs], (((1,), (1,)), ((), ())),
                                            preferred_element_type=F32)
        return acc

    x = x_ref[...].astype(F32).T
    x = attn(x, 0)
    x = ffn(x, True)
    x = attn(x, 1)
    x = ffn(x, False)
    o_ref[...] = x.T.astype(o_ref.dtype)


@jax.jit
def pallas_interleave_layers__sliding_local_dilated__glu_gated_bilinear__prompt_kernel(
        A_x, A_wqkv, A_wo, B_x, B_w_gate, B_w_up, B_w_down):
    Bn, S, _ = A_x.shape
    F = B_w_gate.shape[1]
    nf = F // FC
    x = A_x.reshape(S, D).T
    anyspec = pl.BlockSpec(memory_space=pltpu.HBM)
    out = pl.pallas_call(
        functools.partial(_kernel, nf=nf),
        grid=(S // TM,),
        in_specs=[pl.BlockSpec((D, TM), lambda i: (0, i)),
                  pl.BlockSpec((D, 3 * D), lambda i: (0, 0)),
                  pl.BlockSpec((D, D), lambda i: (0, 0)),
                  anyspec, anyspec, anyspec],
        out_specs=pl.BlockSpec((D, TM), lambda i: (0, i)),
        out_shape=jax.ShapeDtypeStruct((D, S), A_x.dtype),
        scratch_shapes=[pltpu.VMEM((D, 1792), BF), pltpu.VMEM((640, D), BF),
                        pltpu.VMEM((D, F), BF), pltpu.VMEM((D, F), BF), pltpu.VMEM((D, F), BF),
                        pltpu.VMEM((TM + HALO, 1280), F32), pltpu.VMEM((2, HALO, 1280), F32),
                        pltpu.VMEM((TM, 640), BF),
                        pltpu.SemaphoreType.DMA((3, nf))],
        compiler_params=pltpu.CompilerParams(dimension_semantics=("arbitrary",),
                                             vmem_limit_bytes=100 * 1024 * 1024),
    )(x, A_wqkv, A_wo, B_w_gate, B_w_up, B_w_down.T)
    return out.T.reshape(Bn, S, D)
```

```python
import functools
import jax
import jax.numpy as jnp
import jax.experimental.pallas as pl
import jax.experimental.pallas.tpu as pltpu

TM = 512
FC = 2304
UNROLL = 1
DOWN_T = 1
AU = 4
RC = 16
HALO = 16
W, DIL = 8, 2
D, H, DH = 576, 32, 18
BF = jnp.bfloat16
F32 = jnp.float32


def _ln(x):
    m = jnp.mean(x, axis=-1, keepdims=True)
    xc = x - m
    v = jnp.mean(xc * xc, axis=-1, keepdims=True)
    return (xc * jax.lax.rsqrt(v + 1e-5)).astype(BF)


def _kernel(x_ref, wqkv_in, wo_in, wg_hbm, wu_hbm, wd_hbm, o_ref,
            wqkv_ref, wo_ref, wg, wu, wd, kv, halo, obuf, sems, *, nf):
    i = pl.program_id(0)

    def copies(c):
        cs = pl.ds(c * FC, FC)
        return (pltpu.make_async_copy(wg_hbm.at[:, cs], wg.at[:, cs], sems.at[0, c]),
                pltpu.make_async_copy(wu_hbm.at[:, cs], wu.at[:, cs], sems.at[1, c]),
                pltpu.make_async_copy(wd_hbm.at[:, cs], wd.at[:, cs], sems.at[2, c]))

    @pl.when(i == 0)
    def _():
        for c in range(nf):
            for cp in copies(c):
                cp.start()
        halo[...] = jnp.zeros(halo.shape, F32)
        lane = jax.lax.broadcasted_iota(jnp.int32, (640, 128), 1)
        row = jax.lax.broadcasted_iota(jnp.int32, (640, 128), 0)

        def part(sec, n0, lo, hi):
            t0 = {0: 0, 1: 4, 2: 9}[sec] * 128
            n = n0 + lane - lo
            src = (n % H) * DH + n // H + (sec * D - t0)
            ok = (src == row) & (lane >= lo) & (lane < hi)
            wid = min(640, 3 * D - t0)
            P = jnp.where(ok, 1.0, 0.0).astype(BF)[:wid]
            return jnp.dot(wqkv_in[:, t0:t0 + wid], P, preferred_element_type=F32)

        for sec in range(3):
            for j in range(4):
                c = (sec * 4 + j) * 128
                wqkv_ref[:, c:c + 128] = part(sec, j * 128, 0, 128).astype(BF)
        wqkv_ref[:, 1536:1664] = (part(0, 512, 0, 64) + part(2, 512, 64, 128)).astype(BF)
        wqkv_ref[:, 1664:1792] = part(1, 512, 0, 64).astype(BF)
        r = jax.lax.broadcasted_iota(jnp.int32, (640, D), 0)
        cc = jax.lax.broadcasted_iota(jnp.int32, (640, D), 1)
        n = jnp.where(r >= 576, r - 64, r)
        ok = ((n % H) * DH + n // H == cc) & ((r < 512) | (r >= 576))
        wo_ref[...] = jnp.dot(jnp.where(ok, 1.0, 0.0).astype(BF), wo_in[...],
                              preferred_element_type=F32).astype(BF)

    scale = DH ** -0.5

    def attn(x, layer):
        qkv = jnp.dot(_ln(x), wqkv_ref[...], preferred_element_type=F32)
        t = lambda j: qkv[:, j * 128:(j + 1) * 128]
        kv[0:HALO, :] = halo[layer]
        for j in range(4):
            kv[HALO:, j * 128:(j + 1) * 128] = t(4 + j)
            kv[HALO:, (5 + j) * 128:(6 + j) * 128] = t(8 + j)
        kv[HALO:, 512:640] = t(13)
        kv[HALO:, 1152:1280] = t(12)
        halo[layer] = kv[TM:TM + HALO, :]
        for j in range(4):
            kv[HALO:, (10 + j) * 128:(11 + j) * 128] = t(j)

        def rows(r, _):
            r0 = r * RC
            q = [kv[pl.ds(HALO + r0, RC), j * 128:(j + 1) * 128] for j in (10, 11, 12, 13, 9)]
            pos = i * TM + r0 + jax.lax.broadcasted_iota(jnp.int32, (RC, 128), 0)
            lg = []
            for w in range(W):
                s = HALO - DIL * w
                p = None
                for j in range(5):
                    e = q[j] * kv[r0 + s:r0 + s + RC, j * 128:(j + 1) * 128]
                    p = e if p is None else p + e
                p = p + pltpu.roll(p, 64, 1)
                p = (p + pltpu.roll(p, 32, 1)) * scale
                if r0 < DIL * w:
                    p = jnp.where(pos >= DIL * w, p, -1e9)
                lg.append(p)
            m = functools.reduce(jnp.maximum, lg)
            ex = [jnp.exp(p - m) for p in lg]
            inv = 1.0 / functools.reduce(jnp.add, ex)
            for j in range(5):
                acc = None
                for w in range(W):
                    s = HALO - DIL * w
                    e = ex[w] * kv[r0 + s:r0 + s + RC, (5 + j) * 128:(6 + j) * 128]
                    acc = e if acc is None else acc + e
                obuf[pl.ds(r0, RC), j * 128:(j + 1) * 128] = (acc * inv).astype(BF)
        for r in range(TM // RC):
            rows(r, None)
        return x + jnp.dot(obuf[...], wo_ref[...], preferred_element_type=F32)

    def ffn(x, layer):
        xn = _ln(x)

        def body(c, acc):
            @pl.when((i == 0) & (layer == 0))
            def _():
                for cp in copies(c):
                    cp.wait()
            cs = pl.ds(pl.multiple_of(c * FC, FC), FC)
            g = jnp.dot(xn, wg[:, cs], preferred_element_type=F32)
            u = jnp.dot(xn, wu[:, cs], preferred_element_type=F32)
            h = (g * u).astype(BF)
            if DOWN_T:
                return acc + jax.lax.dot_general(wd[:, cs], h, (((1,), (1,)), ((), ())),
                                                 preferred_element_type=F32)
            return acc + jax.lax.dot_general(h, wd[:, cs], (((1,), (1,)), ((), ())),
                                             preferred_element_type=F32)
        if DOWN_T:
            return x + jax.lax.fori_loop(0, nf, body, jnp.zeros((D, TM), F32), unroll=UNROLL).T
        return jax.lax.fori_loop(0, nf, body, x, unroll=UNROLL)

    x = x_ref[...].astype(F32).T
    x = jax.lax.fori_loop(0, 2, lambda l, x: ffn(attn(x, l), l), x)
    o_ref[...] = x.T.astype(o_ref.dtype)


@jax.jit
def pallas_interleave_layers__sliding_local_dilated__glu_gated_bilinear__prompt_kernel(
        A_x, A_wqkv, A_wo, B_x, B_w_gate, B_w_up, B_w_down):
    Bn, S, _ = A_x.shape
    F = B_w_gate.shape[1]
    nf = F // FC
    x = A_x.reshape(S, D).T
    anyspec = pl.BlockSpec(memory_space=pltpu.HBM)
    out = pl.pallas_call(
        functools.partial(_kernel, nf=nf),
        grid=(S // TM,),
        in_specs=[pl.BlockSpec((D, TM), lambda i: (0, i)),
                  pl.BlockSpec((D, 3 * D), lambda i: (0, 0)),
                  pl.BlockSpec((D, D), lambda i: (0, 0)),
                  anyspec, anyspec, anyspec],
        out_specs=pl.BlockSpec((D, TM), lambda i: (0, i)),
        out_shape=jax.ShapeDtypeStruct((D, S), A_x.dtype),
        scratch_shapes=[pltpu.VMEM((D, 1792), BF), pltpu.VMEM((640, D), BF),
                        pltpu.VMEM((D, F), BF), pltpu.VMEM((D, F), BF), pltpu.VMEM((D, F), BF),
                        pltpu.VMEM((TM + HALO, 1792), F32), pltpu.VMEM((2, HALO, 1792), F32),
                        pltpu.VMEM((TM, 640), BF),
                        pltpu.SemaphoreType.DMA((3, nf))],
        compiler_params=pltpu.CompilerParams(dimension_semantics=("arbitrary",),
                                             vmem_limit_bytes=100 * 1024 * 1024),
    )(x, A_wqkv, A_wo, B_w_gate, B_w_up, B_w_down.T)
    return out.T.reshape(Bn, S, D)
```
